```python
import os as _os
_os.environ.setdefault("JAX_PLATFORMS", "cpu")
import jax
import jax.numpy as jnp

def _softmax(x, axis=-1):
    return jax.nn.softmax(x, axis=axis)
def _gelu(x):
    return jax.nn.gelu(x, approximate=True)
def _silu(x):
    return jax.nn.silu(x)
def _sigmoid(x):
    return jax.nn.sigmoid(x)
def _layernorm(x, axis=-1, eps=1e-5):
    m = jnp.mean(x, axis=axis, keepdims=True)
    v = jnp.var(x, axis=axis, keepdims=True)
    return (x - m) / jnp.sqrt(v + eps)
def _scatter_add(tgt, idx, src, axis=0):
    return tgt.at[idx].add(src)
def _segment_sum(src, seg, n):
    return jax.ops.segment_sum(src, seg, n)
class _Rng:
    def __init__(self, key):
        self._k = key
    def _next(self):
        self._k, sub = jax.random.split(self._k)
        return sub
    def normal(self, shape):
        return jax.random.normal(self._next(), shape, dtype=jnp.bfloat16)
    def randint(self, lo, hi, shape):
        return jax.random.randint(self._next(), shape, lo, hi, dtype=jnp.int32)
    def uniform(self, shape, lo=0.0, hi=1.0):
        return jax.random.uniform(self._next(), shape, jnp.bfloat16, lo, hi)
    def permutation(self, n):
        return jax.random.permutation(self._next(), n)


kernel_name = 'sequential_preLN__compressed_kv_cla__dense_activation_mish__decode'

def setup_inputs():
    _rng = _Rng(jax.random.key(int.from_bytes(__import__("os").urandom(4), "little")))
    _w = (lambda a: (lambda t: t.astype(jnp.bfloat16) if jnp.issubdtype(t.dtype, jnp.floating) else t)(jnp.asarray(a)))
    def _A_setup():
        B, H, Sq, Sk, D, M = 1, 32, 1, 8192, 128, 512
        Dc = 4 * D
        return {
            "x": _w((lambda *s: _rng.normal(s) * 0.05)(B, Sq, M)),
            "c_kv": _w((lambda *s: _rng.normal(s) * 0.8)(B, Sk, Dc)),
            "w_q": _w((lambda *s: _rng.normal(s) * 0.8)(M, H, D) * (M ** -0.5)),
            "w_uk": _w((lambda *s: _rng.normal(s) * 0.8)(Dc, H, D) * (Dc ** -0.5)),
            "w_uv": _w((lambda *s: _rng.normal(s) * 0.8)(Dc, H, D) * (Dc ** -0.5)),
            "w_o": _w((lambda *s: _rng.normal(s) * 0.8)(H, D, M) * ((H * D) ** -0.5)),
        }
    _A_in = _A_setup()

    def _B_setup():
        B, S, D, F = 1, 1, 512, 1376
        return {
            "x": _w((lambda *s: _rng.normal(s) * 0.05)(B, S, D)),
            "w1": _w((lambda *s: _rng.normal(s) * 0.2)(D, F) * (D ** -0.5)),
            "b1": _w((lambda *s: _rng.normal(s) * 0.05)(F)),
            "w2": _w((lambda *s: _rng.normal(s) * 0.05)(F, D) * (F ** -0.5)),
        }
    _B_in = _B_setup()

    return {
        "A_x": _A_in["x"],
        "A_c_kv": _A_in["c_kv"],
        "A_w_q": _A_in["w_q"],
        "A_w_uk": _A_in["w_uk"],
        "A_w_uv": _A_in["w_uv"],
        "A_w_o": _A_in["w_o"],
        "B_x": _B_in["x"],
        "B_w1": _B_in["w1"],
        "B_b1": _B_in["b1"],
        "B_w2": _B_in["w2"],
    }

def reference(A_x, A_c_kv, A_w_q, A_w_uk, A_w_uv, A_w_o, B_x, B_w1, B_b1, B_w2):
    def _A_ref(x, c_kv, w_q, w_uk, w_uv, w_o):
        B, Sq, M = x.shape[0], x.shape[1], x.shape[2]
        Sk = c_kv.shape[1]
        H, D = w_q.shape[1], w_q.shape[2]
        q = jnp.einsum("bqm,mhd->bhqd", x, w_q)
        k = jnp.einsum("bkc,chd->bhkd", c_kv, w_uk)
        v = jnp.einsum("bkc,chd->bhkd", c_kv, w_uv)
        scores = jnp.einsum("bhqd,bhkd->bhqk", q, k) * (D ** -0.5)
        off = Sk - Sq
        qi = jnp.arange(Sq)[:, None]
        kj = jnp.arange(Sk)[None, :]
        cmask = kj <= (qi + off)
        scores = jnp.where(cmask[None, None], scores, -1e9)
        p = _softmax(scores, axis=-1)
        ctx = jnp.einsum("bhqk,bhkd->bhqd", p, v)
        return jnp.einsum("bhqd,hdm->bqm", ctx, w_o)

    def _B_ref(x, w1, b1, w2):
        h = jnp.einsum("bsd,df->bsf", x, w1) + b1
        sp = jnp.log1p(jnp.exp(-jnp.abs(h))) + jnp.where(h > 0, h, jnp.zeros_like(h))
        act = h * jnp.tanh(sp)
        return jnp.einsum("bsf,fd->bsd", act, w2)

    x = A_x
    h = x + _A_ref(_layernorm(x, axis=-1), A_c_kv, A_w_q, A_w_uk, A_w_uv, A_w_o)
    h2 = h + _B_ref(_layernorm(h, axis=-1), B_w1, B_b1, B_w2)
    return h2
```

```python
import functools
import jax
import jax.numpy as jnp
from jax import lax
import jax.experimental.pallas as pl
import jax.experimental.pallas.tpu as pltpu

H, D, M, DC, SK, F = 32, 128, 512, 512, 8192, 1376
FP = 1408
NSLOT = 4
BK = 1024

def _ln(x):
    m = jnp.mean(x, axis=-1, keepdims=True)
    xc = x - m
    v = jnp.mean(xc * xc, axis=-1, keepdims=True)
    return xc * lax.rsqrt(v + 1e-5)

def _tile(w_ref, g, u):
    return jnp.concatenate([w_ref[128 * g + 32 * j + u] for j in range(4)], axis=0)

def _kernel(x_hbm, ckv_hbm, wq_hbm, wuk_hbm, wuv_hbm, wo_hbm, w1t_hbm, b1_hbm, w2_hbm, o_ref,
            x_v, b1_v, ckv_v, wq_v, wuk_v, wuv_v, wo_v, w1t_v, w2_v, sems):
    f32, bf16 = jnp.float32, jnp.bfloat16
    chunks = []
    for g in range(4):
        chunks.append((wq_hbm.at[pl.ds(128 * g, 128)], wq_v.at[pl.ds(128 * g, 128)]))
    for g in range(4):
        chunks.append((wuk_hbm.at[pl.ds(128 * g, 128)], wuk_v.at[pl.ds(128 * g, 128)]))
    for i in range(SK // BK):
        chunks.append((ckv_hbm.at[0, pl.ds(BK * i, BK)], ckv_v.at[pl.ds(BK * i, BK)]))
    for g in range(4):
        chunks.append((wuv_hbm.at[pl.ds(128 * g, 128)], wuv_v.at[pl.ds(128 * g, 128)]))
    for a in range(4):
        chunks.append((wo_hbm.at[pl.ds(8 * a, 8)], wo_v.at[pl.ds(8 * a, 8)]))
    chunks.append((w1t_hbm, w1t_v.at[pl.ds(0, F)]))
    w2b = [0, 640, 1152, F]
    for i in range(3):
        chunks.append((w2_hbm.at[pl.ds(w2b[i], w2b[i+1] - w2b[i])], w2_v.at[pl.ds(w2b[i], w2b[i+1] - w2b[i])]))
    n = len(chunks)
    def cp(i):
        return pltpu.make_async_copy(chunks[i][0], chunks[i][1], sems.at[i % NSLOT])
    x_cp = pltpu.make_async_copy(x_hbm.at[0], x_v, sems.at[NSLOT])
    b_cp = pltpu.make_async_copy(b1_hbm, b1_v, sems.at[NSLOT + 1])
    x_cp.start()
    for i in range(NSLOT):
        cp(i).start()
    b_cp.start()
    state = {'i': 0}
    def arrive():
        i = state['i']
        cp(i).wait()
        if i + NSLOT < n:
            cp(i + NSLOT).start()
        state['i'] = i + 1

    w1t_v[pl.ds(F, FP - F), :] = jnp.zeros((FP - F, M), bf16)
    w2_v[pl.ds(F, FP - F), :] = jnp.zeros((FP - F, M), bf16)

    row = lax.broadcasted_iota(jnp.int32, (H, 128), 0)
    lane = lax.broadcasted_iota(jnp.int32, (H, 128), 1)
    diag = (lane % 32) == row
    skew = (lane - row) % 32

    def expand_mm(c, w_ref, g, acc):
        dg = pltpu.roll(c, 0, axis=1, stride=1, stride_axis=0)
        for u in range(32):
            r = dg if u == 0 else pltpu.roll(dg, 128 - u, axis=1)
            s = jnp.where(diag, r, 0.0).astype(bf16)
            acc = acc + jnp.dot(s, _tile(w_ref, g, u), preferred_element_type=f32)
        return acc

    x_cp.wait()
    x = x_v[...].astype(f32)
    xn = _ln(x).astype(bf16).astype(f32)
    xb = jnp.broadcast_to(xn, (H, M))

    q = jnp.zeros((H, D), f32)
    for g in range(4):
        arrive()
        q = expand_mm(xb[:, 128 * g:128 * (g + 1)], wq_v, g, q)
    qb = q.astype(bf16)

    qa = []
    for g in range(4):
        arrive()
        a = jnp.zeros((H, 128), f32)
        for u in range(32):
            y = lax.dot_general(qb, _tile(wuk_v, g, u), (((1,), (1,)), ((), ())), preferred_element_type=f32)
            r = y if u == 0 else pltpu.roll(y, u, axis=1)
            a = jnp.where(skew == u, r, a)
        for b in range(5):
            a = jnp.where((row & (1 << b)) != 0, pltpu.roll(a, 128 - (1 << b), axis=1), a)
        qa.append(a)
    qabs = jnp.concatenate(qa, axis=1).astype(bf16)

    scale = D ** -0.5
    m_run = jnp.full((H, 128), -jnp.inf, f32)
    l_run = jnp.zeros((H, 128), f32)
    acc = jnp.zeros((H, DC), f32)
    for i in range(SK // BK):
        arrive()
        ck = ckv_v[pl.ds(BK * i, BK), :]
        s = lax.dot_general(qabs, ck, (((1,), (1,)), ((), ())), preferred_element_type=f32) * scale
        mx = s[:, 0:128]
        for t in range(1, BK // 128):
            mx = jnp.maximum(mx, s[:, 128 * t:128 * (t + 1)])
        m_new = jnp.maximum(m_run, jnp.max(mx, axis=1, keepdims=True))
        alpha = jnp.exp(m_run - m_new)
        p = jnp.exp(s - m_new[:, 0:1])
        ps = p[:, 0:128]
        for t in range(1, BK // 128):
            ps = ps + p[:, 128 * t:128 * (t + 1)]
        l_run = l_run * alpha + ps
        acc = acc * alpha[:, 0:1] + jnp.dot(p.astype(bf16), ck, preferred_element_type=f32)
        m_run = m_new
    l = jnp.sum(l_run, axis=1, keepdims=True)
    cc = (acc / l).astype(bf16).astype(f32)

    ctx = jnp.zeros((H, D), f32)
    for g in range(4):
        arrive()
        ctx = expand_mm(cc[:, 128 * g:128 * (g + 1)], wuv_v, g, ctx)

    row8 = lax.broadcasted_iota(jnp.int32, (8, 128), 0)
    o8 = jnp.zeros((8, M), f32)
    for a in range(4):
        arrive()
        ca = ctx[8 * a:8 * (a + 1), :]
        la = jnp.concatenate([jnp.where(row8 == r, ca, 0.0) for r in range(8)], axis=1).astype(bf16)
        wa = wo_v[pl.ds(8 * a, 8)].reshape(8 * D, M)
        o8 = o8 + jnp.dot(la, wa, preferred_element_type=f32)
    att = jnp.sum(o8, axis=0, keepdims=True)
    h = (x + att.astype(bf16).astype(f32)).astype(bf16).astype(f32)
    hn = _ln(h).astype(bf16)
    hb = jnp.broadcast_to(hn, (16, M))

    b_cp.wait()
    arrive()
    h1 = lax.dot_general(hb, w1t_v[...], (((1,), (1,)), ((), ())), preferred_element_type=f32)
    h1 = h1[0:8, :]
    b1 = b1_v[...].astype(f32).reshape(1, F)
    b1 = jnp.concatenate([b1, jnp.zeros((1, FP - F), f32)], axis=1)
    z = h1 + b1
    sp = jnp.log1p(jnp.exp(-jnp.abs(z))) + jnp.maximum(z, 0.0)
    act = (z * jnp.tanh(sp)).astype(bf16)
    y = jnp.zeros((8, M), f32)
    w2p = [0, 640, 1152, FP]
    for i in range(3):
        arrive()
        y = y + jnp.dot(act[:, w2p[i]:w2p[i+1]], w2_v[pl.ds(w2p[i], w2p[i+1] - w2p[i]), :], preferred_element_type=f32)
    out = h + y[0:1, :]
    o_ref[0] = out.astype(bf16)


@jax.jit
def pallas_sequential_preLN__compressed_kv_cla__dense_activation_mish__decode_kernel(A_x, A_c_kv, A_w_q, A_w_uk, A_w_uv, A_w_o, B_x, B_w1, B_b1, B_w2):
    vm = pltpu.VMEM
    bf = jnp.bfloat16
    return pl.pallas_call(
        _kernel,
        out_shape=jax.ShapeDtypeStruct((1, 1, M), bf),
        in_specs=[pl.BlockSpec(memory_space=pl.ANY)] * 9,
        out_specs=pl.BlockSpec(memory_space=pltpu.VMEM),
        scratch_shapes=[vm((1, M), bf), vm((F,), bf), vm((SK, DC), bf), vm((M, H, D), bf), vm((DC, H, D), bf),
                        vm((DC, H, D), bf), vm((H, D, M), bf), vm((FP, M), bf), vm((FP, M), bf),
                        pltpu.SemaphoreType.DMA((NSLOT + 2,))],
        compiler_params=pltpu.CompilerParams(vmem_limit_bytes=100 * 1024 * 1024),
    )(A_x, A_c_kv, A_w_q, A_w_uk, A_w_uv, A_w_o, B_w1.T, B_b1, B_w2)
```

```python
import jax
import jax.numpy as jnp
from jax import lax
import jax.experimental.pallas as pl
import jax.experimental.pallas.tpu as pltpu

H, D, M, DC, SK, F = 32, 128, 512, 512, 8192, 1376
FP = 1408
NSLOT = 4
BK = 1024

def _ln(x):
    m = jnp.mean(x, axis=-1, keepdims=True)
    xc = x - m
    v = jnp.mean(xc * xc, axis=-1, keepdims=True)
    return xc * lax.rsqrt(v + 1e-5)

def _tile(w_ref, g, u):
    return jnp.concatenate([w_ref[128 * g + 32 * j + u] for j in range(4)], axis=0)

def _kernel(x_hbm, ckv_hbm, wq_hbm, wuk_hbm, wuv_hbm, wo_hbm, w1t_hbm, b1_hbm, w2_hbm, o_ref,
            x_v, b1_v, ckv_v, wq_v, wuk_v, wuv_v, wo_v, w1t_v, w2_v, sems):
    f32, bf16 = jnp.float32, jnp.bfloat16
    chunks = []
    for g in range(4):
        chunks.append((wq_hbm.at[pl.ds(128 * g, 128)], wq_v.at[pl.ds(128 * g, 128)]))
    for g in range(4):
        chunks.append((wuk_hbm.at[pl.ds(128 * g, 128)], wuk_v.at[pl.ds(128 * g, 128)]))
    for i in range(SK // BK):
        chunks.append((ckv_hbm.at[0, pl.ds(BK * i, BK)], ckv_v.at[pl.ds(BK * i, BK)]))
    for g in range(4):
        chunks.append((wuv_hbm.at[pl.ds(128 * g, 128)], wuv_v.at[pl.ds(128 * g, 128)]))
    for a in range(4):
        chunks.append((wo_hbm.at[pl.ds(8 * a, 8)], wo_v.at[pl.ds(8 * a, 8)]))
    w1b = [0, 384, 768, 1152] + [F]
    for i in range(len(w1b) - 1):
        chunks.append((w1t_hbm.at[pl.ds(w1b[i], w1b[i+1] - w1b[i])], w1t_v.at[pl.ds(w1b[i], w1b[i+1] - w1b[i])]))
    w2b = [0, 384, 768, 1152] + [F]
    for i in range(len(w2b) - 1):
        chunks.append((w2_hbm.at[pl.ds(w2b[i], w2b[i+1] - w2b[i])], w2_v.at[pl.ds(w2b[i], w2b[i+1] - w2b[i])]))
    n = len(chunks)
    def cp(i):
        return pltpu.make_async_copy(chunks[i][0], chunks[i][1], sems.at[i % NSLOT])
    x_cp = pltpu.make_async_copy(x_hbm.at[0], x_v, sems.at[NSLOT])
    b_cp = pltpu.make_async_copy(b1_hbm, b1_v, sems.at[NSLOT])
    x_cp.start()
    b_cp.start()
    for i in range(NSLOT):
        cp(i).start()
    state = {'i': 0}
    def arrive():
        i = state['i']
        cp(i).wait()
        if i + NSLOT < n:
            cp(i + NSLOT).start()
        state['i'] = i + 1

    w1t_v[pl.ds(F, FP - F), :] = jnp.zeros((FP - F, M), bf16)
    w2_v[pl.ds(F, FP - F), :] = jnp.zeros((FP - F, M), bf16)

    row = lax.broadcasted_iota(jnp.int32, (H, 128), 0)
    lane = lax.broadcasted_iota(jnp.int32, (H, 128), 1)
    diag = (lane % 32) == row
    skew = (lane - row) % 32

    def expand_mm(c, w_ref, g, acc):
        dg = c
        for b in range(5):
            dg = jnp.where((row & (1 << b)) != 0, pltpu.roll(dg, 1 << b, axis=1), dg)
        for u in range(32):
            r = dg if u == 0 else pltpu.roll(dg, 128 - u, axis=1)
            s = jnp.where(diag, r, 0.0).astype(bf16)
            acc = acc + jnp.dot(s, _tile(w_ref, g, u), preferred_element_type=f32)
        return acc

    x_cp.wait()
    b_cp.wait()
    x = x_v[...].astype(f32)
    xn = _ln(x).astype(bf16).astype(f32)
    xb = jnp.broadcast_to(xn, (H, M))

    q = jnp.zeros((H, D), f32)
    for g in range(4):
        arrive()
        q = expand_mm(xb[:, 128 * g:128 * (g + 1)], wq_v, g, q)
    qb = q.astype(bf16)

    qa = []
    for g in range(4):
        arrive()
        a = jnp.zeros((H, 128), f32)
        for u in range(32):
            y = lax.dot_general(qb, _tile(wuk_v, g, u), (((1,), (1,)), ((), ())), preferred_element_type=f32)
            r = y if u == 0 else pltpu.roll(y, u, axis=1)
            a = jnp.where(skew == u, r, a)
        for b in range(5):
            a = jnp.where((row & (1 << b)) != 0, pltpu.roll(a, 128 - (1 << b), axis=1), a)
        qa.append(a)
    qabs = jnp.concatenate(qa, axis=1).astype(bf16)

    scale = D ** -0.5
    m_run = jnp.full((H, 128), -jnp.inf, f32)
    l_run = jnp.zeros((H, 128), f32)
    acc = jnp.zeros((H, DC), f32)
    for i in range(SK // BK):
        arrive()
        ck = ckv_v[pl.ds(BK * i, BK), :]
        s = lax.dot_general(qabs, ck, (((1,), (1,)), ((), ())), preferred_element_type=f32) * scale
        mx = s[:, 0:128]
        for t in range(1, BK // 128):
            mx = jnp.maximum(mx, s[:, 128 * t:128 * (t + 1)])
        m_new = jnp.maximum(m_run, jnp.max(mx, axis=1, keepdims=True))
        alpha = jnp.exp(m_run - m_new)
        p = jnp.exp(s - m_new[:, 0:1])
        ps = p[:, 0:128]
        for t in range(1, BK // 128):
            ps = ps + p[:, 128 * t:128 * (t + 1)]
        l_run = l_run * alpha + ps
        acc = acc * alpha[:, 0:1] + jnp.dot(p.astype(bf16), ck, preferred_element_type=f32)
        m_run = m_new
    l = jnp.sum(l_run, axis=1, keepdims=True)
    cc = (acc / l).astype(bf16).astype(f32)

    ctx = jnp.zeros((H, D), f32)
    for g in range(4):
        arrive()
        ctx = expand_mm(cc[:, 128 * g:128 * (g + 1)], wuv_v, g, ctx)

    row8 = lax.broadcasted_iota(jnp.int32, (8, 128), 0)
    o8 = jnp.zeros((8, M), f32)
    for a in range(4):
        arrive()
        ca = ctx[8 * a:8 * (a + 1), :]
        la = jnp.concatenate([jnp.where(row8 == r, ca, 0.0) for r in range(8)], axis=1).astype(bf16)
        wa = wo_v[pl.ds(8 * a, 8)].reshape(8 * D, M)
        o8 = o8 + jnp.dot(la, wa, preferred_element_type=f32)
    att = jnp.sum(o8, axis=0, keepdims=True)
    h = (x + att.astype(bf16).astype(f32)).astype(bf16).astype(f32)
    hn = _ln(h).astype(bf16)
    hb = jnp.broadcast_to(hn, (16, M))

    w1p = w1b[:-1] + [FP]
    parts = []
    for i in range(len(w1b) - 1):
        arrive()
        parts.append(lax.dot_general(hb, w1t_v[pl.ds(w1p[i], w1p[i+1] - w1p[i]), :], (((1,), (1,)), ((), ())),
                                     preferred_element_type=f32)[0:8, :])
    h1 = jnp.concatenate(parts, axis=1)
    b1 = b1_v[...].astype(f32).reshape(1, F)
    b1 = jnp.concatenate([b1, jnp.zeros((1, FP - F), f32)], axis=1)
    z = h1 + b1
    sp = jnp.log1p(jnp.exp(-jnp.abs(z))) + jnp.maximum(z, 0.0)
    act = (z * jnp.tanh(sp)).astype(bf16)
    y = jnp.zeros((8, M), f32)
    w2p = w2b[:-1] + [FP]
    for i in range(len(w2b) - 1):
        arrive()
        y = y + jnp.dot(act[:, w2p[i]:w2p[i+1]], w2_v[pl.ds(w2p[i], w2p[i+1] - w2p[i]), :], preferred_element_type=f32)
    out = h + y[0:1, :]
    o_ref[0] = out.astype(bf16)


@jax.jit
def pallas_sequential_preLN__compressed_kv_cla__dense_activation_mish__decode_kernel(A_x, A_c_kv, A_w_q, A_w_uk, A_w_uv, A_w_o, B_x, B_w1, B_b1, B_w2):
    vm = pltpu.VMEM
    bf = jnp.bfloat16
    return pl.pallas_call(
        _kernel,
        out_shape=jax.ShapeDtypeStruct((1, 1, M), bf),
        in_specs=[pl.BlockSpec(memory_space=pl.ANY)] * 9,
        out_specs=pl.BlockSpec(memory_space=pltpu.VMEM),
        scratch_shapes=[vm((1, M), bf), vm((F,), bf), vm((SK, DC), bf), vm((M, H, D), bf), vm((DC, H, D), bf),
                        vm((DC, H, D), bf), vm((H, D, M), bf), vm((FP, M), bf), vm((FP, M), bf),
                        pltpu.SemaphoreType.DMA((NSLOT + 1,))],
        compiler_params=pltpu.CompilerParams(vmem_limit_bytes=100 * 1024 * 1024),
    )(A_x, A_c_kv, A_w_q, A_w_uk, A_w_uv, A_w_o, B_w1.T, B_b1, B_w2)
```
